```python
import jax
import jax.numpy as jnp

def _softmax(x, axis=-1):
    return jax.nn.softmax(x, axis=axis)

def _gelu(x):
    return jax.nn.gelu(x, approximate=True)

def _silu(x):
    return jax.nn.silu(x)

def _sigmoid(x):
    return jax.nn.sigmoid(x)

def _layernorm(x, axis=-1, eps=1e-05):
    m = jnp.mean(x, axis=axis, keepdims=True)
    v = jnp.var(x, axis=axis, keepdims=True)
    return (x - m) / jnp.sqrt(v + eps)

def _scatter_add(tgt, idx, src, axis=0):
    return tgt.at[idx].add(src)

def _segment_sum(src, seg, n):
    return jax.ops.segment_sum(src, seg, n)

class _Rng:

    def __init__(self, key):
        self._k = key

    def _next(self):
        self._k, sub = jax.random.split(self._k)
        return sub

    def normal(self, shape):
        return jax.random.normal(self._next(), shape, dtype=jnp.bfloat16)

    def randint(self, lo, hi, shape):
        return jax.random.randint(self._next(), shape, lo, hi, dtype=jnp.int32)

    def uniform(self, shape, lo=0.0, hi=1.0):
        return jax.random.uniform(self._next(), shape, jnp.bfloat16, lo, hi)

    def permutation(self, n):
        return jax.random.permutation(self._next(), n)
kernel_name = 'standalone__dilated_atrous__vision'

def setup_inputs():
    _rng = _Rng(jax.random.key(int.from_bytes(__import__("os").urandom(4), "little")))
    _w = lambda a: (lambda t: t.astype(jnp.bfloat16) if jnp.issubdtype(t.dtype, jnp.floating) else t)(jnp.asarray(a))
    H = W = 384
    C = 384
    k = 1
    return {'x': _w((lambda *s: _rng.normal(s) * 0.05)(1, H, W, C)), 'w': _w((lambda *s: _rng.normal(s) * 0.05)(k, k, C, C) * (1.0 / (k * C ** 0.5)))}

def reference(x, w):
    B, H, W, C = x.shape
    k = 1
    rate = 2
    pad = (k - 1) * rate // 2
    xp = jnp.pad(x, ((0, 0), (pad, pad), (pad, pad), (0, 0)))
    out = jnp.zeros_like(x)
    for i in range(k):
        for j in range(k):
            tap = xp[:, i * rate:i * rate + H, j * rate:j * rate + W, :].copy()
            out = out + jnp.einsum('bhwc,co->bhwo', tap, w[i, j])
    return out
```

```python
import jax
import jax.numpy as jnp
from jax import lax
import jax.experimental.pallas as pl
import jax.experimental.pallas.tpu as pltpu

_LANES = 128
_TILE = 8
_SLAB = 4096
_PIECE = 64
_TM = 1024

_R_SLABS = 12
_R_RUN = 2
_LAG = 26
_R_HEAD = 73
_R_STEP = 8
_CUT = 8

_W_SLABS = 6
_W_EARLY = 3
_W_HEAD = 8
_W_STEP = 13


def _split(i, n):
    assert n & (n - 1) == 0
    return lax.shift_right_logical(i, n.bit_length() - 1), i & (n - 1)


@jax.jit
def pallas_standalone__dilated_atrous__vision_kernel(
    x: jax.Array,
    w: jax.Array,
):
    B, H, W, C = x.shape
    assert w.shape == (1, 1, C, C) and C % _LANES == 0
    M = B * H * W
    nc = C // _LANES
    n_slabs = M * nc // _SLAB
    n_steps = M // _TM
    pieces = _SLAB // _PIECE
    assert n_slabs * _SLAB == M * nc and n_steps * _TM == M and _SLAB % _TM == 0

    rounds = _R_SLABS // (2 * _R_RUN)
    n_groups = n_slabs // _R_SLABS
    n_rounds = n_groups * pieces * rounds
    group_steps = _R_SLABS * _SLAB // (nc * _TM)
    assert rounds * 2 * _R_RUN == _R_SLABS and n_groups * _R_SLABS == n_slabs
    assert group_steps * n_groups == n_steps
    cuts = _PIECE // _CUT
    n_cut = pl.cdiv(_LAG, cuts - 1)
    n_cut += -(_LAG + n_cut) % rounds
    tail = _LAG + n_cut
    body = (n_rounds - tail) // rounds
    n1 = (body - _R_HEAD) // _R_STEP
    head = body - n1 * _R_STEP
    assert head >= pieces and tail <= pieces * rounds

    n_writes = n_slabs // _W_SLABS * pieces
    tail_writes = n_cut * cuts - tail + _W_EARLY
    assert n_slabs % _W_SLABS == 0 and tail_writes <= _W_HEAD
    for i in range(n1, n_steps):
        ready = i * nc * _TM // (_W_SLABS * _SLAB) * pieces
        assert _W_HEAD + (i - n1 + 1) * _W_STEP <= ready

    def kernel_function(x_hbm, w_hbm, o_hbm, buf, wbuf):
        def main(read_sems, w_sem, out_sem):
            def read(t, r, queue, line=0, lines=_PIECE):
                g, j = _split(t, pieces)
                slabs = pl.ds(g * _R_SLABS + (2 * r + 1 - queue) * _R_RUN, _R_RUN)
                part = pl.ds(pl.multiple_of(j * _PIECE + line, lines), lines)
                pltpu.make_async_copy(
                    x_hbm.at[slabs, part], buf.at[slabs, part], read_sems.at[g]
                ).start(priority=queue)

            def read_ahead(t, _, first=0, last=rounds):
                for r in range(first, last):
                    read(t + r // rounds, r % rounds, 1)

            def read_sweep(t, _):
                for r in range(rounds):
                    read_ahead(t, None, r + _LAG, r + _LAG + 1)
                    read(t, r, 0)

            def write(t, _=None):
                g, j = _split(t, pieces)
                slabs = pl.ds(g * _W_SLABS, _W_SLABS)
                part = pl.ds(pl.multiple_of(j * _PIECE, _PIECE), _PIECE)
                pltpu.make_async_copy(
                    buf.at[slabs, part], o_hbm.at[slabs, part], out_sem).start()

            def hand_off(k, _):
                def read_round(r, *args):
                    t = lax.div(r, rounds)
                    read(t, r - t * rounds, *args)

                c, p = _split(k, cuts)
                read_round(n_rounds - n_cut + c, 1, p * _CUT, _CUT)
                pl.when(k < tail)(lambda: read_round(n_rounds - tail + k, 0))
                pl.when(k >= tail - _W_EARLY)(lambda: write(k - (tail - _W_EARLY)))

            def step(i, _):
                @pl.when(i < n1)
                def _():
                    t = head + i * _R_STEP
                    lax.fori_loop(0, _R_STEP, lambda a, _: read_sweep(t + a, _), None)

                @pl.when(i == n1)
                def _():
                    lax.fori_loop(0, n_cut * cuts, hand_off, None)
                    lax.fori_loop(tail_writes, _W_HEAD, write, None)

                @pl.when(i >= n1)
                def _():
                    for a in range(_W_STEP):
                        write(_W_HEAD + (i - n1) * _W_STEP + a)

                g, q = _split(i, group_steps)

                @pl.when(q == 0)
                def _():
                    slabs = pl.ds(g * _R_SLABS, _R_SLABS)
                    pltpu.make_async_copy(
                        x_hbm.at[slabs], buf.at[slabs], read_sems.at[g]).wait()

                parts = []
                for c in range(nc):
                    s, line = _split((i * nc + c) * _TM, _SLAB)
                    parts.append((s, pl.ds(pl.multiple_of(line, _TM), _TM)))
                tiles = jnp.concatenate([buf[p] for p in parts], axis=0)
                tiles = tiles.reshape(_TM // _TILE, nc, _TILE, _LANES)
                xv = jnp.concatenate(
                    [tiles[:, c].reshape(_TM, _LANES) for c in range(nc)], axis=1)
                res = jnp.dot(xv, wbuf[...], preferred_element_type=jnp.float32)
                tiles = jnp.stack(
                    [res[:, c * _LANES:(c + 1) * _LANES].reshape(-1, _TILE, _LANES)
                     for c in range(nc)], axis=1)
                lines = tiles.reshape(nc * _TM, _LANES).astype(buf.dtype)
                for c, p in enumerate(parts):
                    buf[p] = lines[c * _TM:(c + 1) * _TM]

            w_copy = pltpu.make_async_copy(w_hbm, wbuf, w_sem)
            w_copy.start()
            lax.fori_loop(0, _LAG // rounds, read_ahead, None)
            read_ahead(jnp.int32(_LAG // rounds), None, 0, _LAG % rounds)
            lax.fori_loop(0, head, read_sweep, None)
            w_copy.wait()

            lax.fori_loop(0, n_steps, step, None)

            lax.fori_loop(_W_HEAD + (n_steps - n1) * _W_STEP, n_writes, write, None)
            pltpu.make_async_copy(buf, o_hbm, out_sem).wait()

        pl.run_scoped(
            main,
            pltpu.SemaphoreType.DMA((n_groups,)),
            pltpu.SemaphoreType.DMA(()),
            pltpu.SemaphoreType.DMA(()),
        )

    x_lines = x.reshape(M // _TILE, _TILE, nc, _LANES).transpose(0, 2, 1, 3)
    out = pl.pallas_call(
        kernel_function,
        in_specs=[
            pl.BlockSpec(memory_space=pl.ANY),
            pl.BlockSpec(memory_space=pl.ANY),
        ],
        out_specs=pl.BlockSpec(memory_space=pl.ANY),
        out_shape=jax.ShapeDtypeStruct((n_slabs, _SLAB, _LANES), x.dtype),
        scratch_shapes=[
            pltpu.VMEM((n_slabs, _SLAB, _LANES), x.dtype),
            pltpu.VMEM((C, C), w.dtype),
        ],
        compiler_params=pltpu.CompilerParams(
            vmem_limit_bytes=120 * 2**20, disable_bounds_checks=True),
    )(x_lines.reshape(n_slabs, _SLAB, _LANES), w.reshape(C, C))
    out = out.reshape(M // _TILE, nc, _TILE, _LANES).transpose(0, 2, 1, 3)
    return out.reshape(B, H, W, C)
```

```python
import jax
import jax.numpy as jnp
from jax import lax
import jax.experimental.pallas as pl
import jax.experimental.pallas.tpu as pltpu

_LANES = 128
_TILE = 8
_SLAB = 4096
_PIECE = 64
_TM = 1024

_R_SLABS = 12
_R_RUN = (1, 3)
_LAG = 9
_R_HEAD = 70
_R_STEP = 8
_SHORT = _PIECE // 4

_W_SLABS = 6
_W_HEAD = 20
_W_STEP = 13


def _split(i, n):
    assert n & (n - 1) == 0
    return lax.shift_right_logical(i, n.bit_length() - 1), i & (n - 1)


@jax.jit
def pallas_standalone__dilated_atrous__vision_kernel(
    x: jax.Array,
    w: jax.Array,
):
    B, H, W, C = x.shape
    assert w.shape == (1, 1, C, C) and C % _LANES == 0
    M = B * H * W
    nc = C // _LANES
    n_slabs = M * nc // _SLAB
    n_steps = M // _TM
    pieces = _SLAB // _PIECE
    assert n_slabs * _SLAB == M * nc and n_steps * _TM == M and _SLAB % _TM == 0

    rounds = _R_SLABS // sum(_R_RUN)
    n_groups = n_slabs // _R_SLABS
    assert rounds * sum(_R_RUN) == _R_SLABS and n_groups * _R_SLABS == n_slabs
    last = n_groups * pieces - 1
    cuts = _R_RUN[1] * _PIECE // _SHORT
    body = last - _LAG
    assert cuts > _LAG
    n1 = (body - _R_HEAD) // _R_STEP
    head = body - n1 * _R_STEP
    group_steps = pieces // _R_STEP
    assert head >= pieces and group_steps * (n_groups - 1) >= n1
    assert group_steps * nc * _TM <= _R_SLABS * _SLAB

    n_writes = n_slabs // _W_SLABS * pieces
    assert n_slabs % _W_SLABS == 0
    for i in range(n1, n_steps):
        ready = i * nc * _TM // (_W_SLABS * _SLAB) * pieces
        assert _W_HEAD + (i - n1 + 1) * _W_STEP <= ready

    def kernel_function(x_hbm, w_hbm, o_hbm, buf, wbuf):
        def main(read_sems, w_sem, out_sem):
            def read(queue, t, r, cut=None):
                g, j = _split(t, pieces)
                slab = g * _R_SLABS + r * sum(_R_RUN) + (0 if queue else _R_RUN[1])
                if cut is None:
                    slabs = pl.ds(slab, _R_RUN[queue])
                    part = pl.ds(pl.multiple_of(j * _PIECE, _PIECE), _PIECE)
                else:
                    s, p = _split(cut, _PIECE // _SHORT)
                    slabs = slab + s
                    part = pl.ds(pl.multiple_of(j * _PIECE + p * _SHORT, _SHORT), _SHORT)
                pltpu.make_async_copy(
                    x_hbm.at[slabs, part], buf.at[slabs, part], read_sems.at[g]
                ).start(priority=queue)

            def fill_queue(t, _):
                for r in range(rounds):
                    read(1, t, r)

            def read_sweep(t, _=None):
                for r in range(rounds):
                    read(1, t + _LAG, r)
                    read(0, t, r)

            def read_tail(k, _):
                for r in range(rounds):
                    read(1, jnp.int32(last), r, k)
                    pl.when(k <= _LAG)(lambda: read(0, body + k, r))

            def write(t, _=None):
                g, j = _split(t, pieces)
                slabs = pl.ds(g * _W_SLABS, _W_SLABS)
                part = pl.ds(pl.multiple_of(j * _PIECE, _PIECE), _PIECE)
                pltpu.make_async_copy(
                    buf.at[slabs, part], o_hbm.at[slabs, part], out_sem).start()

            def step(i, _):
                @pl.when(i < n1)
                def _():
                    t = head + i * _R_STEP
                    lax.fori_loop(0, _R_STEP, lambda a, _: read_sweep(t + a), None)

                @pl.when(i == n1)
                def _():
                    lax.fori_loop(0, cuts, read_tail, None)
                    lax.fori_loop(0, _W_HEAD, write, None)

                @pl.when(i >= n1)
                def _():
                    for a in range(_W_STEP):
                        write(_W_HEAD + (i - n1) * _W_STEP + a)

                g, q = _split(i, group_steps)

                @pl.when((q == 0) & (g < n_groups))
                def _():
                    slabs = pl.ds(g * _R_SLABS, _R_SLABS)
                    pltpu.make_async_copy(
                        x_hbm.at[slabs], buf.at[slabs], read_sems.at[g]).wait()

                parts = []
                for c in range(nc):
                    s, line = _split((i * nc + c) * _TM, _SLAB)
                    parts.append((s, pl.ds(pl.multiple_of(line, _TM), _TM)))
                tiles = jnp.concatenate([buf[p] for p in parts], axis=0)
                tiles = tiles.reshape(_TM // _TILE, nc, _TILE, _LANES)
                xv = jnp.concatenate(
                    [tiles[:, c].reshape(_TM, _LANES) for c in range(nc)], axis=1)
                res = jnp.dot(xv, wbuf[...], preferred_element_type=jnp.float32)
                tiles = jnp.stack(
                    [res[:, c * _LANES:(c + 1) * _LANES].reshape(-1, _TILE, _LANES)
                     for c in range(nc)], axis=1)
                lines = tiles.reshape(nc * _TM, _LANES).astype(buf.dtype)
                for c, p in enumerate(parts):
                    buf[p] = lines[c * _TM:(c + 1) * _TM]

            w_copy = pltpu.make_async_copy(w_hbm, wbuf, w_sem)
            w_copy.start()
            lax.fori_loop(0, _LAG, fill_queue, None)
            lax.fori_loop(0, head, read_sweep, None)
            w_copy.wait()

            lax.fori_loop(0, n_steps, step, None)

            lax.fori_loop(_W_HEAD + (n_steps - n1) * _W_STEP, n_writes, write, None)
            pltpu.make_async_copy(buf, o_hbm, out_sem).wait()

        pl.run_scoped(
            main,
            pltpu.SemaphoreType.DMA((n_groups,)),
            pltpu.SemaphoreType.DMA(()),
            pltpu.SemaphoreType.DMA(()),
        )

    x_lines = x.reshape(M // _TILE, _TILE, nc, _LANES).transpose(0, 2, 1, 3)
    out = pl.pallas_call(
        kernel_function,
        in_specs=[
            pl.BlockSpec(memory_space=pl.ANY),
            pl.BlockSpec(memory_space=pl.ANY),
        ],
        out_specs=pl.BlockSpec(memory_space=pl.ANY),
        out_shape=jax.ShapeDtypeStruct((n_slabs, _SLAB, _LANES), x.dtype),
        scratch_shapes=[
            pltpu.VMEM((n_slabs, _SLAB, _LANES), x.dtype),
            pltpu.VMEM((C, C), w.dtype),
        ],
        compiler_params=pltpu.CompilerParams(
            vmem_limit_bytes=120 * 2**20, disable_bounds_checks=True),
    )(x_lines.reshape(n_slabs, _SLAB, _LANES), w.reshape(C, C))
    out = out.reshape(M // _TILE, nc, _TILE, _LANES).transpose(0, 2, 1, 3)
    return out.reshape(B, H, W, C)
```

```python
import jax
import jax.numpy as jnp
from jax import lax
import jax.experimental.pallas as pl
import jax.experimental.pallas.tpu as pltpu

_LANES = 128
_TILE = 8
_SLAB = 4096
_PIECE = 64
_TM = 1024

_R_SLABS = 12
_R_RUN = (1, 3)
_LAG = 9
_R_HEAD = 70
_R_STEP = 8
_SHORT = _PIECE // 4

_W_SLABS = 6
_W_HEAD = 20
_W_STEP = 13


def _split(i, n):
    assert n & (n - 1) == 0
    return lax.shift_right_logical(i, n.bit_length() - 1), i & (n - 1)


@jax.jit
def pallas_standalone__dilated_atrous__vision_kernel(
    x: jax.Array,
    w: jax.Array,
):
    B, H, W, C = x.shape
    assert w.shape == (1, 1, C, C) and C % _LANES == 0
    M = B * H * W
    nc = C // _LANES
    n_slabs = M * nc // _SLAB
    n_steps = M // _TM
    pieces = _SLAB // _PIECE
    assert n_slabs * _SLAB == M * nc and n_steps * _TM == M and _SLAB % _TM == 0

    rounds = _R_SLABS // sum(_R_RUN)
    n_groups = n_slabs // _R_SLABS
    assert rounds * sum(_R_RUN) == _R_SLABS and n_groups * _R_SLABS == n_slabs
    last = n_groups * pieces - 1
    cuts = _R_RUN[1] * _PIECE // _SHORT
    body = last - _LAG
    assert cuts > _LAG
    n1 = (body - _R_HEAD) // _R_STEP
    head = body - n1 * _R_STEP
    group_steps = pieces // _R_STEP
    assert head >= pieces and group_steps * (n_groups - 1) >= n1
    assert group_steps * nc * _TM <= _R_SLABS * _SLAB

    n_writes = n_slabs // _W_SLABS * pieces
    assert n_slabs % _W_SLABS == 0
    for i in range(n1, n_steps):
        ready = i * nc * _TM // (_W_SLABS * _SLAB) * pieces
        assert _W_HEAD + (i - n1 + 1) * _W_STEP <= ready

    def kernel_function(x_hbm, w_hbm, o_hbm, buf, wbuf):
        def main(read_sems, w_sem, out_sem):
            def read(queue, t, r, cut=None):
                g, j = _split(t, pieces)
                slab = g * _R_SLABS + r * sum(_R_RUN) + (0 if queue else _R_RUN[1])
                if cut is None:
                    slabs = pl.ds(slab, _R_RUN[queue])
                    part = pl.ds(pl.multiple_of(j * _PIECE, _PIECE), _PIECE)
                else:
                    s, p = _split(cut, _PIECE // _SHORT)
                    slabs = slab + s
                    part = pl.ds(pl.multiple_of(j * _PIECE + p * _SHORT, _SHORT), _SHORT)
                pltpu.make_async_copy(
                    x_hbm.at[slabs, part], buf.at[slabs, part], read_sems.at[g]
                ).start(priority=queue)

            def fill_queue(t, _):
                for r in range(rounds):
                    read(1, t, r)

            def read_sweep(t, _=None):
                for r in range(rounds):
                    read(1, t + _LAG, r)
                    read(0, t, r)

            def read_tail(k, _):
                for r in range(rounds):
                    read(1, jnp.int32(last), r, k)
                    pl.when(k <= _LAG)(lambda: read(0, body + k, r))

            def write(t, _=None):
                g, j = _split(t, pieces)
                slabs = pl.ds(g * _W_SLABS, _W_SLABS)
                part = pl.ds(pl.multiple_of(j * _PIECE, _PIECE), _PIECE)
                pltpu.make_async_copy(
                    buf.at[slabs, part], o_hbm.at[slabs, part], out_sem).start()

            def step(i, _):
                @pl.when(i < n1)
                def _():
                    t = head + jnp.minimum(i, n1 - 1) * _R_STEP
                    lax.fori_loop(0, _R_STEP, lambda a, _: read_sweep(t + a), None)

                @pl.when(i == n1)
                def _():
                    lax.fori_loop(0, cuts, read_tail, None)
                    lax.fori_loop(0, _W_HEAD, write, None)

                @pl.when(i >= n1)
                def _():
                    for a in range(_W_STEP):
                        write(_W_HEAD + jnp.maximum(i - n1, 0) * _W_STEP + a)

                g, q = _split(i, group_steps)

                @pl.when((q == 0) & (g < n_groups))
                def _():
                    slabs = pl.ds(g * _R_SLABS, _R_SLABS)
                    pltpu.make_async_copy(
                        x_hbm.at[slabs], buf.at[slabs], read_sems.at[g]).wait()

                parts = []
                for c in range(nc):
                    s, line = _split((i * nc + c) * _TM, _SLAB)
                    parts.append((s, pl.ds(pl.multiple_of(line, _TM), _TM)))
                tiles = jnp.concatenate([buf[p] for p in parts], axis=0)
                tiles = tiles.reshape(_TM // _TILE, nc, _TILE, _LANES)
                xv = jnp.concatenate(
                    [tiles[:, c:c + 1].reshape(_TM, _LANES) for c in range(nc)], axis=1)
                res = jnp.dot(xv, wbuf[...], preferred_element_type=jnp.float32)
                tiles = jnp.concatenate(
                    [res[:, c * _LANES:(c + 1) * _LANES].reshape(-1, _TILE, _LANES)
                     for c in range(nc)], axis=1)
                lines = tiles.reshape(nc * _TM, _LANES).astype(buf.dtype)
                for c, p in enumerate(parts):
                    buf[p] = lines[c * _TM:(c + 1) * _TM]

            w_copy = pltpu.make_async_copy(w_hbm, wbuf, w_sem)
            w_copy.start()
            lax.fori_loop(0, _LAG, fill_queue, None)
            lax.fori_loop(0, head, read_sweep, None)
            w_copy.wait()

            lax.fori_loop(0, n_steps, step, None)

            lax.fori_loop(_W_HEAD + (n_steps - n1) * _W_STEP, n_writes, write, None)
            pltpu.make_async_copy(buf, o_hbm, out_sem).wait()

        pl.run_scoped(
            main,
            pltpu.SemaphoreType.DMA((n_groups,)),
            pltpu.SemaphoreType.DMA(()),
            pltpu.SemaphoreType.DMA(()),
        )

    x_lines = x.reshape(M // _TILE, _TILE, nc, _LANES).transpose(0, 2, 1, 3)
    out = pl.pallas_call(
        kernel_function,
        in_specs=[
            pl.BlockSpec(memory_space=pl.ANY),
            pl.BlockSpec(memory_space=pl.ANY),
        ],
        out_specs=pl.BlockSpec(memory_space=pl.ANY),
        out_shape=jax.ShapeDtypeStruct((n_slabs, _SLAB, _LANES), x.dtype),
        scratch_shapes=[
            pltpu.VMEM((n_slabs, _SLAB, _LANES), x.dtype),
            pltpu.VMEM((C, C), w.dtype),
        ],
        compiler_params=pltpu.CompilerParams(vmem_limit_bytes=120 * 2**20),
    )(x_lines.reshape(n_slabs, _SLAB, _LANES), w.reshape(C, C))
    out = out.reshape(M // _TILE, nc, _TILE, _LANES).transpose(0, 2, 1, 3)
    return out.reshape(B, H, W, C)
```
